```python
import os as _os
_os.environ.setdefault("JAX_PLATFORMS", "cpu")
import jax
import jax.numpy as jnp

def _softmax(x, axis=-1):
    return jax.nn.softmax(x, axis=axis)
def _gelu(x):
    return jax.nn.gelu(x, approximate=True)
def _silu(x):
    return jax.nn.silu(x)
def _sigmoid(x):
    return jax.nn.sigmoid(x)
def _layernorm(x, axis=-1, eps=1e-5):
    m = jnp.mean(x, axis=axis, keepdims=True)
    v = jnp.var(x, axis=axis, keepdims=True)
    return (x - m) / jnp.sqrt(v + eps)
def _scatter_add(tgt, idx, src, axis=0):
    return tgt.at[idx].add(src)
def _segment_sum(src, seg, n):
    return jax.ops.segment_sum(src, seg, n)
class _Rng:
    def __init__(self, key):
        self._k = key
    def _next(self):
        self._k, sub = jax.random.split(self._k)
        return sub
    def normal(self, shape):
        return jax.random.normal(self._next(), shape, dtype=jnp.bfloat16)
    def randint(self, lo, hi, shape):
        return jax.random.randint(self._next(), shape, lo, hi, dtype=jnp.int32)
    def uniform(self, shape, lo=0.0, hi=1.0):
        return jax.random.uniform(self._next(), shape, jnp.bfloat16, lo, hi)
    def permutation(self, n):
        return jax.random.permutation(self._next(), n)


kernel_name = 'concat_heads__mha_block_cached__mha_block_cached__near_ridge'

def setup_inputs():
    _rng = _Rng(jax.random.key(int.from_bytes(__import__("os").urandom(4), "little")))
    _w = (lambda a: (lambda t: t.astype(jnp.bfloat16) if jnp.issubdtype(t.dtype, jnp.floating) else t)(jnp.asarray(a)))
    def _A_setup():
        B, Sq, D = 16, 80, 512
        H, Sk, Dh = 32, 80, 128
        return {
            "x": _w((lambda *s: _rng.normal(s) * 0.8)(B, Sq, D)),
            "k_cache": _w((lambda *s: _rng.normal(s) * 0.8)(B, H, Sk, Dh)),
            "v_cache": _w((lambda *s: _rng.normal(s) * 0.05)(B, H, Sk, Dh)),
            "wq": _w((lambda *s: _rng.normal(s) * 0.8)(D, H * Dh) * (D ** -0.5)),
            "wo": _w((lambda *s: _rng.normal(s) * 0.05)(H * Dh, D) * ((H * Dh) ** -0.5)),
        }
    _A_in = _A_setup()

    def _B_setup():
        B, Sq, D = 16, 80, 512
        H, Sk, Dh = 32, 80, 128
        return {
            "x": _w((lambda *s: _rng.normal(s) * 0.8)(B, Sq, D)),
            "k_cache": _w((lambda *s: _rng.normal(s) * 0.8)(B, H, Sk, Dh)),
            "v_cache": _w((lambda *s: _rng.normal(s) * 0.05)(B, H, Sk, Dh)),
            "wq": _w((lambda *s: _rng.normal(s) * 0.8)(D, H * Dh) * (D ** -0.5)),
            "wo": _w((lambda *s: _rng.normal(s) * 0.05)(H * Dh, D) * ((H * Dh) ** -0.5)),
        }
    _B_in = _B_setup()

    return {
        "A_x": _A_in["x"],
        "A_k_cache": _A_in["k_cache"],
        "A_v_cache": _A_in["v_cache"],
        "A_wq": _A_in["wq"],
        "A_wo": _A_in["wo"],
        "B_x": _B_in["x"],
        "B_k_cache": _B_in["k_cache"],
        "B_v_cache": _B_in["v_cache"],
        "B_wq": _B_in["wq"],
        "B_wo": _B_in["wo"],
    }

def reference(A_x, A_k_cache, A_v_cache, A_wq, A_wo, B_x, B_k_cache, B_v_cache, B_wq, B_wo):
    def _A_ref(x, k_cache, v_cache, wq, wo):
        B, Sq, D = x.shape
        H, Dh = 32, 128
        q = (lambda x, *d: x.transpose(*d))((x @ wq).reshape(B, Sq, H, Dh), 0, 2, 1, 3)
        scores = jnp.einsum("bhqd,bhkd->bhqk", q, k_cache) * (Dh ** -0.5)
        p = _softmax(scores, axis=-1)
        o = jnp.einsum("bhqk,bhkd->bhqd", p, v_cache)
        return (lambda x, *d: x.transpose(*d))(o, 0, 2, 1, 3).reshape(B, Sq, H * Dh) @ wo

    def _B_ref(x, k_cache, v_cache, wq, wo):
        B, Sq, D = x.shape
        H, Dh = 32, 128
        q = (lambda x, *d: x.transpose(*d))((x @ wq).reshape(B, Sq, H, Dh), 0, 2, 1, 3)
        scores = jnp.einsum("bhqd,bhkd->bhqk", q, k_cache) * (Dh ** -0.5)
        p = _softmax(scores, axis=-1)
        o = jnp.einsum("bhqk,bhkd->bhqd", p, v_cache)
        return (lambda x, *d: x.transpose(*d))(o, 0, 2, 1, 3).reshape(B, Sq, H * Dh) @ wo

    a = _A_ref(A_x, A_k_cache, A_v_cache, A_wq, A_wo)
    b = _B_ref(B_x, B_k_cache, B_v_cache, B_wq, B_wo)
    return jnp.concatenate([a, b], axis=-1)
```

```python
import functools, math
import jax, jax.numpy as jnp
from jax import lax
from jax.experimental import pallas as pl
from jax.experimental.pallas import tpu as pltpu

B, S, D, H, Dh = 16, 80, 512, 32, 128
M = B * S
C = (Dh ** -0.5) * math.log2(math.e)
HQ = 4
QH = H // HQ
NQ = 2 * QH
CB = 4
NC = B // CB
R = CB * S
NSLOT = 4


def make(rcp='approx', vmem=110, nobc=True, nodma=False):

    def recip(l):
        r = pl.reciprocal(l, approx=True)
        if rcp == 'newton':
            r = r * (2.0 - l * r)
        return r

    def kern(ax, ak, av, awq, awo, bx, bk, bv, bwq, bwo, out,
             x_buf, kv_buf, wq_buf, wo_buf, q_scr, o_scr, acc, stage,
             sem_x, sem_h, sem_kv, sem_wq, sem_wo, sem_out):

        class Dummy:
            def start(self): pass
            def wait(self): pass
        def cp(src, dst, sem):
            if nodma: return Dummy()
            return pltpu.make_async_copy(src, dst, sem)

        def rows(c):
            return slice(c * R, (c + 1) * R)

        def xa_copy(c):
            return cp(ax.at[rows(c)], x_buf.at[0, rows(c)], sem_x.at[c])
        def xb_copy():
            return cp(bx, x_buf.at[1], sem_x.at[NC])
        def wq0_first():
            return cp(awq.at[:, 0:Dh], wq_buf.at[0, :, 0:Dh], sem_h.at[0])
        def wq0_rest():
            return cp(awq.at[:, Dh:HQ * Dh], wq_buf.at[0, :, Dh:HQ * Dh], sem_h.at[1])
        def pair_copies(p):
            return [cp(ak.at[:, pl.ds(2 * p, 2)], kv_buf.at[0, 0, :, pl.ds(2 * p, 2)], sem_h.at[2 + 4 * p]),
                    cp(av.at[:, pl.ds(2 * p, 2)], kv_buf.at[0, 1, :, pl.ds(2 * p, 2)], sem_h.at[3 + 4 * p]),
                    cp(awo.at[pl.ds(2 * p * Dh, 2 * Dh), :], wo_buf.at[0, pl.ds(2 * p * Dh, 2 * Dh), :], sem_h.at[4 + 4 * p]),
                    cp(awq.at[:, pl.ds((HQ + 2 * p) * Dh, 2 * Dh)], wq_buf.at[1, :, pl.ds(2 * p * Dh, 2 * Dh)], sem_h.at[5 + 4 * p])]

        def by_half(q, fn):
            if isinstance(q, int):
                if q < QH: fn(0, q)
                elif q < NQ: fn(1, q - QH)
                return
            @pl.when(q < QH)
            def _(): fn(0, q)
            @pl.when(jnp.logical_and(q >= QH, q < NQ))
            def _(): fn(1, q - QH)

        def slot_of(q):
            return q % NSLOT if isinstance(q, int) else lax.bitwise_and(q, NSLOT - 1)

        def start_kvo(q):
            sl = slot_of(q)
            def fn(half, g):
                cp((ak, bk)[half].at[:, pl.ds(g * HQ, HQ)], kv_buf.at[sl, 0], sem_kv.at[sl]).start()
                cp((av, bv)[half].at[:, pl.ds(g * HQ, HQ)], kv_buf.at[sl, 1], sem_kv.at[sl]).start()
                cp((awo, bwo)[half].at[pl.ds(g * (HQ * Dh), HQ * Dh), :], wo_buf.at[sl], sem_wo.at[sl]).start()
            by_half(q, fn)
        def start_wq(q):
            sl = slot_of(q)
            by_half(q, lambda half, g: cp((awq, bwq)[half].at[:, pl.ds(g * (HQ * Dh), HQ * Dh)], wq_buf.at[sl], sem_wq.at[sl]).start())
        def wait_kvo(q):
            sl = slot_of(q)
            cp(kv_buf.at[sl], kv_buf.at[sl], sem_kv.at[sl]).wait()
            cp(wo_buf.at[sl], wo_buf.at[sl], sem_wo.at[sl]).wait()
        def wait_wq(q):
            sl = slot_of(q)
            cp(wq_buf.at[sl], wq_buf.at[sl], sem_wq.at[sl]).wait()

        def half_of(q):
            return int(q >= QH) if isinstance(q, int) else jnp.where(q >= QH, 1, 0)

        def qproj(sx, wsl, i, c, qsl):
            q_scr[qsl, i, rows(c), :] = jnp.dot(x_buf[sx, rows(c), :], wq_buf[wsl, :, pl.ds(i * Dh, Dh)],
                                                preferred_element_type=jnp.float32).astype(jnp.bfloat16)
        def oproj_val(osl, wsl, i, c):
            return jnp.dot(o_scr[osl, rows(c), :], wo_buf[wsl, pl.ds(i * Dh, Dh), :], preferred_element_type=jnp.float32)
        def scores(qsl, kvsl, i, c):
            q = q_scr[qsl, i, rows(c), :].reshape(CB, S, Dh)
            k = kv_buf[kvsl, 0, c * CB:(c + 1) * CB, i]
            sc = jnp.einsum('bqd,bkd->bqk', q, k, preferred_element_type=jnp.float32)
            m = jnp.max(sc, axis=-1, keepdims=True)
            p = jnp.exp2((sc - m) * C)
            l = jnp.sum(p, axis=-1, keepdims=True)
            return p.astype(jnp.bfloat16), l
        def pv(pb, l, osl, kvsl, i, c):
            v = kv_buf[kvsl, 1, c * CB:(c + 1) * CB, i]
            o = jnp.einsum('bqk,bkd->bqd', pb, v, preferred_element_type=jnp.float32)
            o = o * recip(l)
            o_scr[osl, rows(c), :] = o.astype(jnp.bfloat16).reshape(R, Dh)

        def body(items):
            n = len(items)
            def do_o(it):
                qsl, kvsl, i, c, sa = it['att']
                acc[sa, rows(c), :] += oproj_val(0, kvsl, i, c)
            def do_q(it):
                if it['q'] is not None: qproj(*it['q'])
            for j, it in enumerate(items):
                qsl, kvsl, i, c, sa = it['att']
                pb, l = scores(qsl, kvsl, i, c)
                if j < n - 1:
                    do_q(it)
                    pv(pb, l, 0, kvsl, i, c)
                    if j > 0: do_o(items[j - 1])
                else:
                    do_o(items[j - 1])
                    pv(pb, l, 0, kvsl, i, c)
                    do_q(it)
                    do_o(it)

        def ordered(thunks):
            def bd(i, c):
                lax.switch(i, [(lambda th=th: th()) for th in thunks])
                return c
            lax.fori_loop(0, len(thunks), bd, 0)
        def st(*cps):
            def th():
                for c_ in cps: c_.start()
            return th
        ordered([st(wq0_first(), xa_copy(0)), st(wq0_rest(), xa_copy(1))])
        acc[...] = jnp.zeros_like(acc)

        wq0_first().wait()
        xa_copy(0).wait()
        xa_copy(2).start(); xa_copy(3).start()
        qproj(0, 0, 0, 0, 0)
        wq0_rest().wait()
        for c_ in pair_copies(0): c_.start()
        for i in range(1, HQ): qproj(0, 0, i, 0, 0)
        xa_copy(1).wait()
        for c_ in pair_copies(1): c_.start()
        for i in range(HQ): qproj(0, 0, i, 1, 0)
        xa_copy(2).wait()
        start_kvo(1); start_wq(2)
        for i in range(HQ): qproj(0, 0, i, 2, 0)
        xa_copy(3).wait()
        start_kvo(2); start_wq(3)
        for i in range(HQ): qproj(0, 0, i, 3, 0)
        start_kvo(3); start_wq(4)
        xb_copy().start()

        def pair_body(p, carry):
            qd = lax.shift_right_logical(p, 1)
            hf = lax.bitwise_and(p, 1)
            @pl.when(p < 2)
            def _():
                for c_ in pair_copies(p): c_.wait()
            @pl.when(jnp.logical_and(p >= 2, hf == 0))
            def _():
                wait_kvo(qd); wait_wq(qd + 1)
            qsl = lax.bitwise_and(qd, 1)
            items = []
            for ii in range(2):
                for c in range(NC):
                    i = 2 * hf + ii
                    items.append(dict(att=(qsl, qd, i, c, 0), q=(0, qd + 1, i, c, 1 - qsl)))
            body(items)
            @pl.when(hf == 1)
            def _():
                start_kvo(qd + NSLOT); start_wq(qd + 1 + NSLOT)
            return carry
        lax.fori_loop(0, 6, pair_body, 0)

        def main_body(m, carry):
            q0 = 3 + 2 * m
            @pl.when(q0 + 1 == QH)
            def _():
                xb_copy().wait()
            wait_kvo(q0); wait_kvo(q0 + 1); wait_wq(q0 + 1); wait_wq(q0 + 2)
            items = []
            for d in range(2):
                qq = q0 + d
                sl = slot_of(qq); sln = slot_of(qq + 1)
                sa = half_of(qq); sx = half_of(qq + 1)
                for i in range(HQ):
                    for c in range(NC):
                        items.append(dict(att=((1 + d) % 2, sl, i, c, sa), q=(sx, sln, i, c, d % 2)))
            body(items)
            start_kvo(q0 + NSLOT); start_kvo(q0 + 1 + NSLOT)
            start_wq(q0 + 1 + NSLOT); start_wq(q0 + 2 + NSLOT)
            return carry
        lax.fori_loop(0, 6, main_body, 0)

        ql = NQ - 1
        sl = ql % NSLOT
        qsl = ql % 2
        wait_kvo(ql)
        stage[0] = acc[0].astype(jnp.bfloat16)
        pltpu.make_async_copy(stage.at[0], out.at[:, pl.ds(0, D)], sem_out.at[NC]).start()
        def fin_o(osl, i, c):
            if i == HQ - 1:
                val = acc[1, rows(c), :] + oproj_val(osl, sl, i, c)
                stage[1, rows(c), :] = val.astype(jnp.bfloat16)
                pltpu.make_async_copy(stage.at[1, rows(c)], out.at[rows(c), pl.ds(D, D)], sem_out.at[c]).start()
            else:
                acc[1, rows(c), :] += oproj_val(osl, sl, i, c)
        prev = None
        for j in range(HQ * NC):
            c, i = divmod(j, HQ)
            pb, l = scores(qsl, sl, i, c)
            if prev is not None:
                fin_o(*prev)
            pv(pb, l, j % 2, sl, i, c)
            prev = (j % 2, i, c)
        fin_o(*prev)
        for c in range(NC):
            pltpu.make_async_copy(stage.at[1, rows(c)], out.at[rows(c), pl.ds(D, D)], sem_out.at[c]).wait()
        pltpu.make_async_copy(stage.at[0], out.at[:, pl.ds(0, D)], sem_out.at[NC]).wait()

    @jax.jit
    def f(A_x, A_k, A_v, A_wq, A_wo, B_x, B_k, B_v, B_wq, B_wo):
        any_spec = pl.BlockSpec(memory_space=pl.ANY)
        o = pl.pallas_call(
            kern,
            in_specs=[any_spec] * 10,
            out_specs=any_spec,
            out_shape=jax.ShapeDtypeStruct((M, 2 * D), jnp.bfloat16),
            scratch_shapes=[
                pltpu.VMEM((2, M, D), jnp.bfloat16),
                pltpu.VMEM((NSLOT, 2, B, HQ, S, Dh), jnp.bfloat16),
                pltpu.VMEM((NSLOT, D, HQ * Dh), jnp.bfloat16),
                pltpu.VMEM((NSLOT, HQ * Dh, D), jnp.bfloat16),
                pltpu.VMEM((2, HQ, M, Dh), jnp.bfloat16),
                pltpu.VMEM((2, M, Dh), jnp.bfloat16),
                pltpu.VMEM((2, M, D), jnp.float32),
                pltpu.VMEM((2, M, D), jnp.bfloat16),
                pltpu.SemaphoreType.DMA((NC + 1,)),
                pltpu.SemaphoreType.DMA((10,)),
                pltpu.SemaphoreType.DMA((NSLOT,)), pltpu.SemaphoreType.DMA((NSLOT,)), pltpu.SemaphoreType.DMA((NSLOT,)),
                pltpu.SemaphoreType.DMA((NC + 1,)),
            ],
            compiler_params=pltpu.CompilerParams(vmem_limit_bytes=vmem * 1024 * 1024, disable_bounds_checks=nobc),
        )(A_x.reshape(M, D), A_k, A_v, A_wq, A_wo, B_x.reshape(M, D), B_k, B_v, B_wq, B_wo)
        return o.reshape(B, S, 2 * D)
    return f


_impl = make()


@jax.jit
def pallas_concat_heads__mha_block_cached__mha_block_cached__near_ridge_kernel(
    A_x: jax.Array,
    A_k_cache: jax.Array,
    A_v_cache: jax.Array,
    A_wq: jax.Array,
    A_wo: jax.Array,
    B_x: jax.Array,
    B_k_cache: jax.Array,
    B_v_cache: jax.Array,
    B_wq: jax.Array,
    B_wo: jax.Array,
):
    return _impl(A_x, A_k_cache, A_v_cache, A_wq, A_wo, B_x, B_k_cache, B_v_cache, B_wq, B_wo)
```

```python
import functools, math
import jax, jax.numpy as jnp
from jax import lax
from jax.experimental import pallas as pl
from jax.experimental.pallas import tpu as pltpu

B, S, D, H, Dh = 16, 80, 512, 32, 128
M = B * S
C = (Dh ** -0.5) * math.log2(math.e)
HQ = 4
QH = H // HQ
NQ = 2 * QH
CB = 4
NC = B // CB
R = CB * S
NSLOT = 4


def make(rcp='approx', vmem=110, nodma=False, merge23=False, tail_split=2, scopes=False, last_order='deep', use_first=True, use_stage=True, dummy_zero=False, unroll_ramp=True):

    def recip(l):
        r = pl.reciprocal(l, approx=True)
        if rcp == 'newton':
            r = r * (2.0 - l * r)
        return r

    class NoScope:
        def __enter__(self): return self
        def __exit__(self, *a): return False
    def scope(name):
        return jax.named_scope(name) if scopes else NoScope()

    def kern(ax, ak, av, awq, awo, bx, bk, bv, bwq, bwo, out,
             x_buf, kv_buf, wq_buf, wo_buf, q_scr, o_scr, acc, stage,
             sem_pro, sem_kv, sem_wq, sem_wo, sem_out):

        class Dummy:
            def start(self): pass
            def wait(self): pass
        def cp(src, dst, sem):
            if nodma: return Dummy()
            return pltpu.make_async_copy(src, dst, sem)

        def rows(c):
            return slice(c * R, (c + 1) * R)

        def xa_copy(c):
            return cp(ax.at[rows(c)], x_buf.at[0, rows(c)], sem_pro.at[c])
        def xb_copy():
            return cp(bx, x_buf.at[1], sem_pro.at[0])
        def wq0_first():
            return cp(awq.at[:, 0:Dh], wq_buf.at[0, :, 0:Dh], sem_pro.at[4])
        def wq0_rest():
            return cp(awq.at[:, Dh:HQ * Dh], wq_buf.at[0, :, Dh:HQ * Dh], sem_pro.at[5])
        def pair_copies(p):
            return [cp(ak.at[:, pl.ds(2 * p, 2)], kv_buf.at[0, 0, :, pl.ds(2 * p, 2)], sem_pro.at[6 + 4 * p]),
                    cp(av.at[:, pl.ds(2 * p, 2)], kv_buf.at[0, 1, :, pl.ds(2 * p, 2)], sem_pro.at[7 + 4 * p]),
                    cp(awo.at[pl.ds(2 * p * Dh, 2 * Dh), :], wo_buf.at[0, pl.ds(2 * p * Dh, 2 * Dh), :], sem_pro.at[8 + 4 * p]),
                    cp(awq.at[:, pl.ds((HQ + 2 * p) * Dh, 2 * Dh)], wq_buf.at[1, :, pl.ds(2 * p * Dh, 2 * Dh)], sem_pro.at[9 + 4 * p])]

        def by_half(q, fn):
            if isinstance(q, int):
                if q < QH: fn(0, q)
                elif q < NQ: fn(1, q - QH)
                return
            @pl.when(q < QH)
            def _(): fn(0, q)
            @pl.when(jnp.logical_and(q >= QH, q < NQ))
            def _(): fn(1, q - QH)

        def slot_of(q):
            return q % NSLOT if isinstance(q, int) else lax.bitwise_and(q, NSLOT - 1)

        def start_kvo(q):
            sl = slot_of(q)
            def fn(half, g):
                cp((ak, bk)[half].at[:, pl.ds(g * HQ, HQ)], kv_buf.at[sl, 0], sem_kv.at[sl]).start()
                cp((av, bv)[half].at[:, pl.ds(g * HQ, HQ)], kv_buf.at[sl, 1], sem_kv.at[sl]).start()
                cp((awo, bwo)[half].at[pl.ds(g * (HQ * Dh), HQ * Dh), :], wo_buf.at[sl], sem_wo.at[sl]).start()
            by_half(q, fn)
        def start_wq(q):
            sl = slot_of(q)
            by_half(q, lambda half, g: cp((awq, bwq)[half].at[:, pl.ds(g * (HQ * Dh), HQ * Dh)], wq_buf.at[sl], sem_wq.at[sl]).start())
        def wait_kvo(q):
            sl = slot_of(q)
            cp(kv_buf.at[sl], kv_buf.at[sl], sem_kv.at[sl]).wait()
            cp(wo_buf.at[sl], wo_buf.at[sl], sem_wo.at[sl]).wait()
        def wait_wq(q):
            sl = slot_of(q)
            cp(wq_buf.at[sl], wq_buf.at[sl], sem_wq.at[sl]).wait()

        def half_of(q):
            return int(q >= QH) if isinstance(q, int) else jnp.where(q >= QH, 1, 0)

        def qproj(sx, wsl, i, c, qsl):
            q_scr[qsl, i, rows(c), :] = jnp.dot(x_buf[sx, rows(c), :], wq_buf[wsl, :, pl.ds(i * Dh, Dh)],
                                                preferred_element_type=jnp.float32).astype(jnp.bfloat16)
        def oproj_val(osl, wsl, i, r0, n):
            return jnp.dot(o_scr[osl, r0:r0 + n, :], wo_buf[wsl, pl.ds(i * Dh, Dh), :], preferred_element_type=jnp.float32)
        def scores(qsl, kvsl, i, c):
            q = q_scr[qsl, i, rows(c), :].reshape(CB, S, Dh)
            k = kv_buf[kvsl, 0, c * CB:(c + 1) * CB, i]
            sc = lax.dot_general(q, k, (((2,), (2,)), ((0,), (0,))), preferred_element_type=jnp.float32)
            m = jnp.max(sc, axis=-1, keepdims=True)
            p = jnp.exp2((sc - m) * C)
            l = jnp.sum(p, axis=-1, keepdims=True)
            return p.astype(jnp.bfloat16), l
        def pv(pb, l, osl, kvsl, i, c):
            v = kv_buf[kvsl, 1, c * CB:(c + 1) * CB, i]
            o = lax.dot_general(pb, v, (((2,), (1,)), ((0,), (0,))), preferred_element_type=jnp.float32)
            o = o * recip(l)
            o_scr[osl, rows(c), :] = o.astype(jnp.bfloat16).reshape(R, Dh)

        def do_o(it, osl):
            qsl, kvsl, i, c, sa = it['att']
            if it.get('final'):
                nsp = tail_split if c == NC - 1 else 1
                n = R // nsp
                for k in range(nsp):
                    r0 = c * R + k * n
                    val = acc[sa, r0:r0 + n, :] + oproj_val(osl, kvsl, i, r0, n)
                    stage[sa, r0:r0 + n, :] = val.astype(jnp.bfloat16)
                    cpy = pltpu.make_async_copy(stage.at[sa, r0:r0 + n], out.at[r0:r0 + n, pl.ds(D, D)], sem_out.at[1 + c + k])
                    cpy.start()
                    it['copies'].append(cpy)
                return
            val = oproj_val(osl, kvsl, i, c * R, R)
            first = it.get('first') if use_first else None
            if first is None:
                val = acc[sa, rows(c), :] + val
            elif first is True:
                pass
            else:
                val = jnp.where(first, 0.0, acc[sa, rows(c), :]) + val
            acc[sa, rows(c), :] = val
            if it.get('stage') and use_stage:
                stage[sa, rows(c), :] = val.astype(jnp.bfloat16)

        def do_q(it):
            if it['q'] is not None: qproj(*it['q'])

        def body(items):
            n = len(items)
            nq = sum(1 for it in items if it['q'] is not None)
            sc = {}
            def S_(j):
                qsl, kvsl, i, c, sa = items[j]['att']
                sc[j] = scores(qsl, kvsl, i, c)
            def P_(j):
                qsl, kvsl, i, c, sa = items[j]['att']
                pb, l = sc.pop(j)
                pv(pb, l, j % 2, kvsl, i, c)
            def O_(j):
                do_o(items[j], j % 2)
            if nq == n:
                for j in range(n):
                    S_(j)
                    if j < n - 1:
                        do_q(items[j]); P_(j)
                        if j > 0: O_(j - 1)
                    else:
                        O_(j - 1); P_(j); do_q(items[j]); O_(j)
            else:
                for j in range(nq):
                    S_(j); do_q(items[j]); P_(j)
                    if j > 0: O_(j - 1)
                if last_order == 'deep':
                    S_(nq)
                    if nq > 0: O_(nq - 1)
                    for j in range(nq, n):
                        if j + 1 < n: S_(j + 1)
                        P_(j)
                        if j > nq: O_(j - 1)
                    O_(n - 1)
                else:
                    for j in range(nq, n):
                        S_(j)
                        if j > 0: O_(j - 1)
                        P_(j)
                    O_(n - 1)

        def ordered(thunks):
            def bd(i, c):
                lax.switch(i, [(lambda th=th: th()) for th in thunks])
                return c
            lax.fori_loop(0, len(thunks), bd, 0)
        def st(*cps):
            def th():
                for c_ in cps: c_.start()
            return th
        with scope('issue0'):
            ordered([st(wq0_first(), xa_copy(0)), st(wq0_rest(), xa_copy(1))])
        with scope('w0'):
            wq0_first().wait()
            xa_copy(0).wait()
        xa_copy(2).start(); xa_copy(3).start()
        qproj(0, 0, 0, 0, 0)
        with scope('w1'):
            wq0_rest().wait()
        start_wq(1)
        for i in range(1, HQ): qproj(0, 0, i, 0, 0)
        with scope('w2'):
            xa_copy(1).wait()
        start_kvo(0)
        for i in range(HQ): qproj(0, 0, i, 1, 0)
        with scope('w3'):
            xa_copy(2).wait(); xa_copy(3).wait()
        start_wq(2)
        for c in (2, 3):
            for i in range(HQ): qproj(0, 0, i, c, 0)
        with scope('w4'):
            wait_wq(1)
        start_kvo(1); start_wq(3); start_kvo(2)
        for c in range(NC):
            for i in range(HQ): qproj(0, 1, i, c, 1)
        start_kvo(3); start_wq(4); start_wq(5)

        def quad_body(r, carry):
            with scope('wquad'):
                wait_kvo(r); wait_wq(r + 2)
            items = [dict(att=(r, r, i, c, 0), q=(0, r + 2, i, c, r + 2), first=(r == 0) if i == 0 else None)
                     for i in range(HQ) for c in range(NC)]
            with scope('quadbody'):
                body(items)
                start_kvo(r + NSLOT); start_wq(r + 2 + NSLOT)
            return carry
        with scope('ramp'):
            lax.fori_loop(0, 2, quad_body, 0)

        def main_body(m, carry):
            q0 = 2 + 2 * m
            @pl.when(q0 + 2 == QH)
            def _():
                xb_copy().wait()
            wait_kvo(q0); wait_kvo(q0 + 1); wait_wq(q0 + 2); wait_wq(q0 + 3)
            @pl.when(q0 == QH)
            def _():
                pltpu.make_async_copy(stage.at[0], out.at[:, pl.ds(0, D)], sem_out.at[0]).start()
            items = []
            for d in range(2):
                qq = q0 + d
                sl = slot_of(qq); sln = slot_of(qq + 2)
                sa = half_of(qq); sx = half_of(qq + 2)
                for i in range(HQ):
                    for c in range(NC):
                        items.append(dict(att=(sl, sl, i, c, sa), q=(sx, sln, i, c, sln),
                                          first=(qq == QH) if (d == 0 and i == 0) else None,
                                          stage=(d == 1 and i == HQ - 1)))
            with scope('mainbody'):
                body(items)
                start_kvo(q0 + NSLOT); start_kvo(q0 + 1 + NSLOT)
                start_wq(q0 + 2 + NSLOT); start_wq(q0 + 3 + NSLOT)
                @pl.when(m == 0)
                def _():
                    xb_copy().start()
            return carry
        with scope('main'):
            lax.fori_loop(0, 6, main_body, 0)

        with scope('wlast'):
            wait_kvo(NQ - 2); wait_kvo(NQ - 1)
        copies = []
        s14, s15 = (NQ - 2) % NSLOT, (NQ - 1) % NSLOT
        items = [dict(att=(s14, s14, i, c, 1), q=None) for i in range(HQ) for c in range(NC)]
        items += [dict(att=(s15, s15, i, c, 1), q=None, final=(i == HQ - 1), copies=copies) for c in range(NC) for i in range(HQ)]
        body(items)
        with scope('wout'):
            for cpy in copies: cpy.wait()
            pltpu.make_async_copy(stage.at[0], out.at[:, pl.ds(0, D)], sem_out.at[0]).wait()

    @jax.jit
    def f(A_x, A_k, A_v, A_wq, A_wo, B_x, B_k, B_v, B_wq, B_wo):
        any_spec = pl.BlockSpec(memory_space=pl.ANY)
        o = pl.pallas_call(
            kern,
            in_specs=[any_spec] * 10,
            out_specs=any_spec,
            out_shape=jax.ShapeDtypeStruct((M, 2 * D), jnp.bfloat16),
            scratch_shapes=[
                pltpu.VMEM((2, M, D), jnp.bfloat16),
                pltpu.VMEM((NSLOT, 2, B, HQ, S, Dh), jnp.bfloat16),
                pltpu.VMEM((NSLOT, D, HQ * Dh), jnp.bfloat16),
                pltpu.VMEM((NSLOT, HQ * Dh, D), jnp.bfloat16),
                pltpu.VMEM((NSLOT, HQ, M, Dh), jnp.bfloat16),
                pltpu.VMEM((2, M, Dh), jnp.bfloat16),
                pltpu.VMEM((2, M, D), jnp.float32),
                pltpu.VMEM((2, M, D), jnp.bfloat16),
                pltpu.SemaphoreType.DMA((14,)),
                pltpu.SemaphoreType.DMA((NSLOT,)), pltpu.SemaphoreType.DMA((NSLOT,)), pltpu.SemaphoreType.DMA((NSLOT,)),
                pltpu.SemaphoreType.DMA((NC + tail_split,)),
            ],
            compiler_params=pltpu.CompilerParams(vmem_limit_bytes=vmem * 1024 * 1024, disable_bounds_checks=True,
                                                 disable_semaphore_checks=True),
        )(A_x.reshape(M, D), A_k, A_v, A_wq, A_wo, B_x.reshape(M, D), B_k, B_v, B_wq, B_wo)
        return o.reshape(B, S, 2 * D)
    return f


_impl = make()


@jax.jit
def pallas_concat_heads__mha_block_cached__mha_block_cached__near_ridge_kernel(
    A_x: jax.Array,
    A_k_cache: jax.Array,
    A_v_cache: jax.Array,
    A_wq: jax.Array,
    A_wo: jax.Array,
    B_x: jax.Array,
    B_k_cache: jax.Array,
    B_v_cache: jax.Array,
    B_wq: jax.Array,
    B_wo: jax.Array,
):
    return _impl(A_x, A_k_cache, A_v_cache, A_wq, A_wo, B_x, B_k_cache, B_v_cache, B_wq, B_wo)
```

```python
import math
import jax, jax.numpy as jnp
from jax import lax
from jax.experimental import pallas as pl
from jax.experimental.pallas import tpu as pltpu

B, S, D, H, Dh = 16, 80, 512, 32, 128
M = B * S
C = (Dh ** -0.5) * math.log2(math.e)
HQ = 4
QH = H // HQ
NQ = 2 * QH
XC = 4
XR = M // XC
NSLOT = 4


def make(cb_main=8, cb_ramp=8, last_chunks=(4, 4, 4, 4), last14=8, tail_pieces=(80, 80, 80, 80), vmem=110, scopes=False):

    class NoScope:
        def __enter__(self): return self
        def __exit__(self, *a): return False
    def scope(name):
        return jax.named_scope(name) if scopes else NoScope()

    def chunks(sizes):
        out, b0 = [], 0
        for n in sizes:
            out.append((b0, n)); b0 += n
        assert b0 == B
        return out
    def even(cb):
        return chunks([cb] * (B // cb))

    n_out_sems = 1 + len(last_chunks) + len(tail_pieces)
    assert sum(tail_pieces) == last_chunks[-1] * S

    def kern(ax, ak, av, awq, awo, bx, bk, bv, bwq, bwo, out,
             x_buf, kv_buf, wq_buf, wo_buf, q_scr, o_scr, acc, stage,
             sem_pro, sem_kv, sem_wq, sem_wo, sem_out):

        cp = pltpu.make_async_copy

        def rows(ch):
            b0, nb = ch
            return slice(b0 * S, (b0 + nb) * S)

        def xa_copy(c):
            return cp(ax.at[c * XR:(c + 1) * XR], x_buf.at[0, c * XR:(c + 1) * XR], sem_pro.at[c])
        def xb_copy():
            return cp(bx, x_buf.at[1], sem_pro.at[0])
        def wq0_first():
            return cp(awq.at[:, 0:Dh], wq_buf.at[0, :, 0:Dh], sem_pro.at[4])
        def wq0_rest():
            return cp(awq.at[:, Dh:HQ * Dh], wq_buf.at[0, :, Dh:HQ * Dh], sem_pro.at[5])

        def by_half(q, fn):
            if isinstance(q, int):
                if q < QH: fn(0, q)
                elif q < NQ: fn(1, q - QH)
                return
            @pl.when(q < QH)
            def _(): fn(0, q)
            @pl.when(jnp.logical_and(q >= QH, q < NQ))
            def _(): fn(1, q - QH)

        def slot_of(q):
            return q % NSLOT if isinstance(q, int) else lax.bitwise_and(q, NSLOT - 1)

        def start_kvo(q):
            sl = slot_of(q)
            def fn(half, g):
                cp((ak, bk)[half].at[:, pl.ds(g * HQ, HQ)], kv_buf.at[sl, 0], sem_kv.at[sl]).start()
                cp((av, bv)[half].at[:, pl.ds(g * HQ, HQ)], kv_buf.at[sl, 1], sem_kv.at[sl]).start()
                cp((awo, bwo)[half].at[pl.ds(g * (HQ * Dh), HQ * Dh), :], wo_buf.at[sl], sem_wo.at[sl]).start()
            by_half(q, fn)
        def start_wq(q):
            sl = slot_of(q)
            by_half(q, lambda half, g: cp((awq, bwq)[half].at[:, pl.ds(g * (HQ * Dh), HQ * Dh)], wq_buf.at[sl], sem_wq.at[sl]).start())
        def wait_kvo(q):
            sl = slot_of(q)
            cp(kv_buf.at[sl], kv_buf.at[sl], sem_kv.at[sl]).wait()
            cp(wo_buf.at[sl], wo_buf.at[sl], sem_wo.at[sl]).wait()
        def wait_wq(q):
            sl = slot_of(q)
            cp(wq_buf.at[sl], wq_buf.at[sl], sem_wq.at[sl]).wait()

        def half_of(q):
            return int(q >= QH) if isinstance(q, int) else jnp.where(q >= QH, 1, 0)

        def qproj(sx, wsl, i, rs, qsl):
            q_scr[qsl, i, rs, :] = jnp.dot(x_buf[sx, rs, :], wq_buf[wsl, :, pl.ds(i * Dh, Dh)],
                                           preferred_element_type=jnp.float32).astype(jnp.bfloat16)
        def oproj_val(osl, wsl, i, rs):
            return jnp.dot(o_scr[osl, rs, :], wo_buf[wsl, pl.ds(i * Dh, Dh), :], preferred_element_type=jnp.float32)
        def scores(sl, i, ch):
            b0, nb = ch
            q = q_scr[sl, i, rows(ch), :].reshape(nb, S, Dh)
            k = kv_buf[sl, 0, b0:b0 + nb, i]
            sc = lax.dot_general(q, k, (((2,), (2,)), ((0,), (0,))), preferred_element_type=jnp.float32)
            m = jnp.max(sc, axis=-1, keepdims=True)
            p = jnp.exp2((sc - m) * C)
            l = jnp.sum(p, axis=-1, keepdims=True)
            return p.astype(jnp.bfloat16), l
        def pv(pb, l, osl, sl, i, ch):
            b0, nb = ch
            v = kv_buf[sl, 1, b0:b0 + nb, i]
            o = lax.dot_general(pb, v, (((2,), (1,)), ((0,), (0,))), preferred_element_type=jnp.float32)
            o = o * pl.reciprocal(l, approx=True)
            o_scr[osl, rows(ch), :] = o.astype(jnp.bfloat16).reshape(nb * S, Dh)

        def do_o(it, osl):
            sl, i, ch, sa = it['att']
            rs = rows(ch)
            if it.get('final'):
                pieces = tail_pieces if it['final'] == 'split' else (rs.stop - rs.start,)
                r0 = rs.start
                for n in pieces:
                    r = slice(r0, r0 + n)
                    r0 += n
                    val = acc[sa, r, :] + oproj_val(osl, sl, i, r)
                    stage[sa, r, :] = val.astype(jnp.bfloat16)
                    cpy = cp(stage.at[sa, r], out.at[r, pl.ds(D, D)], sem_out.at[1 + len(it['copies'])])
                    cpy.start()
                    it['copies'].append(cpy)
                return
            val = oproj_val(osl, sl, i, rs)
            first = it.get('first')
            if first is None:
                val = acc[sa, rs, :] + val
            else:
                val = jnp.where(first, 0.0, acc[sa, rs, :]) + val
            acc[sa, rs, :] = val
            if it.get('stage'):
                stage[sa, rs, :] = val.astype(jnp.bfloat16)

        def body(items):
            n = len(items)
            with_q = items[0]['q'] is not None
            sc = {}
            def S_(j):
                sl, i, ch, sa = items[j]['att']
                sc[j] = scores(sl, i, ch)
            def P_(j):
                sl, i, ch, sa = items[j]['att']
                pb, l = sc.pop(j)
                pv(pb, l, j % 2, sl, i, ch)
            def O_(j):
                do_o(items[j], j % 2)
            def Q_(j):
                qproj(*items[j]['q'])
            if with_q:
                for j in range(n):
                    S_(j)
                    if j < n - 1:
                        Q_(j); P_(j)
                        if j > 0: O_(j - 1)
                    else:
                        O_(j - 1); P_(j); Q_(j); O_(j)
            else:
                S_(0)
                for j in range(n):
                    if j + 1 < n: S_(j + 1)
                    P_(j)
                    if j > 0: O_(j - 1)
                O_(n - 1)

        def ordered(thunks):
            def bd(i, c):
                lax.switch(i, thunks)
                return c
            lax.fori_loop(0, len(thunks), bd, 0)
        def st(*cps):
            def th():
                for c_ in cps: c_.start()
            return th
        def xr(c0, c1):
            return slice(c0 * XR, c1 * XR)
        with scope('issue0'):
            ordered([st(wq0_first(), xa_copy(0)), st(wq0_rest(), xa_copy(1))])
        with scope('w0'):
            wq0_first().wait()
            xa_copy(0).wait()
        xa_copy(2).start(); xa_copy(3).start()
        qproj(0, 0, 0, xr(0, 1), 0)
        with scope('w1'):
            wq0_rest().wait()
        start_wq(1)
        for i in range(1, HQ): qproj(0, 0, i, xr(0, 1), 0)
        with scope('w2'):
            xa_copy(1).wait(); xa_copy(2).wait()
        start_kvo(0); start_wq(2)
        for c in (1, 2):
            for i in range(HQ): qproj(0, 0, i, xr(c, c + 1), 0)
        with scope('w3'):
            xa_copy(3).wait(); wait_wq(1)
        start_kvo(1); start_wq(3); start_kvo(2)
        for i in range(HQ): qproj(0, 0, i, xr(3, 4), 0)
        for c in range(XC):
            for i in range(HQ): qproj(0, 1, i, xr(c, c + 1), 1)
        start_kvo(3); start_wq(4); start_wq(5)

        def quad_body(r, carry):
            with scope('wquad'):
                wait_kvo(r); wait_wq(r + 2)
            items = [dict(att=(r, i, ch, 0), q=(0, r + 2, i, rows(ch), r + 2), first=(r == 0) if i == 0 else None)
                     for i in range(HQ) for ch in even(cb_ramp)]
            with scope('quadbody'):
                body(items)
                start_kvo(r + NSLOT); start_wq(r + 2 + NSLOT)
            return carry
        with scope('ramp'):
            lax.fori_loop(0, 2, quad_body, 0)

        def main_body(m, carry):
            q0 = 2 + 2 * m
            @pl.when(q0 + 2 == QH)
            def _():
                xb_copy().wait()
            wait_kvo(q0); wait_kvo(q0 + 1); wait_wq(q0 + 2); wait_wq(q0 + 3)
            @pl.when(q0 == QH)
            def _():
                cp(stage.at[0], out.at[:, pl.ds(0, D)], sem_out.at[0]).start()
            items = []
            for d in range(2):
                qq = q0 + d
                sl = slot_of(qq); sln = slot_of(qq + 2)
                sa = half_of(qq); sx = half_of(qq + 2)
                for i in range(HQ):
                    for ch in even(cb_main):
                        items.append(dict(att=(sl, i, ch, sa), q=(sx, sln, i, rows(ch), sln),
                                          first=(qq == QH) if (d == 0 and i == 0) else None,
                                          stage=(d == 1 and i == HQ - 1)))
            with scope('mainbody'):
                body(items)
                start_kvo(q0 + NSLOT); start_kvo(q0 + 1 + NSLOT)
                start_wq(q0 + 2 + NSLOT); start_wq(q0 + 3 + NSLOT)
                @pl.when(m == 0)
                def _():
                    xb_copy().start()
            return carry
        with scope('main'):
            lax.fori_loop(0, 6, main_body, 0)

        with scope('wlast'):
            wait_kvo(NQ - 2); wait_kvo(NQ - 1)
        copies = []
        s14, s15 = (NQ - 2) % NSLOT, (NQ - 1) % NSLOT
        items = [dict(att=(s14, i, ch, 1), q=None) for i in range(HQ) for ch in even(last14)]
        lc = chunks(list(last_chunks))
        for k, ch in enumerate(lc):
            for i in range(HQ):
                fin = None
                if i == HQ - 1:
                    fin = 'split' if k == len(lc) - 1 else 'whole'
                items.append(dict(att=(s15, i, ch, 1), q=None, final=fin, copies=copies))
        body(items)
        with scope('wout'):
            for cpy in copies: cpy.wait()
            cp(stage.at[0], out.at[:, pl.ds(0, D)], sem_out.at[0]).wait()

    @jax.jit
    def f(A_x, A_k, A_v, A_wq, A_wo, B_x, B_k, B_v, B_wq, B_wo):
        any_spec = pl.BlockSpec(memory_space=pl.ANY)
        o = pl.pallas_call(
            kern,
            in_specs=[any_spec] * 10,
            out_specs=any_spec,
            out_shape=jax.ShapeDtypeStruct((M, 2 * D), jnp.bfloat16),
            scratch_shapes=[
                pltpu.VMEM((2, M, D), jnp.bfloat16),
                pltpu.VMEM((NSLOT, 2, B, HQ, S, Dh), jnp.bfloat16),
                pltpu.VMEM((NSLOT, D, HQ * Dh), jnp.bfloat16),
                pltpu.VMEM((NSLOT, HQ * Dh, D), jnp.bfloat16),
                pltpu.VMEM((NSLOT, HQ, M, Dh), jnp.bfloat16),
                pltpu.VMEM((2, M, Dh), jnp.bfloat16),
                pltpu.VMEM((2, M, D), jnp.float32),
                pltpu.VMEM((2, M, D), jnp.bfloat16),
                pltpu.SemaphoreType.DMA((6,)),
                pltpu.SemaphoreType.DMA((NSLOT,)), pltpu.SemaphoreType.DMA((NSLOT,)), pltpu.SemaphoreType.DMA((NSLOT,)),
                pltpu.SemaphoreType.DMA((n_out_sems,)),
            ],
            compiler_params=pltpu.CompilerParams(vmem_limit_bytes=vmem * 1024 * 1024, disable_bounds_checks=True,
                                                 disable_semaphore_checks=True),
        )(A_x.reshape(M, D), A_k, A_v, A_wq, A_wo, B_x.reshape(M, D), B_k, B_v, B_wq, B_wo)
        return o.reshape(B, S, 2 * D)
    return f


_impl = make(last_chunks=(4,4,4,2,2),tail_pieces=(96,48,16))


@jax.jit
def pallas_concat_heads__mha_block_cached__mha_block_cached__near_ridge_kernel(
    A_x: jax.Array,
    A_k_cache: jax.Array,
    A_v_cache: jax.Array,
    A_wq: jax.Array,
    A_wo: jax.Array,
    B_x: jax.Array,
    B_k_cache: jax.Array,
    B_v_cache: jax.Array,
    B_wq: jax.Array,
    B_wo: jax.Array,
):
    return _impl(A_x, A_k_cache, A_v_cache, A_wq, A_wo, B_x, B_k_cache, B_v_cache, B_wq, B_wo)
```

```python
import math

import jax
import jax.numpy as jnp
from jax import lax
from jax.experimental import pallas as pl
from jax.experimental.pallas import tpu as pltpu

B, S, D, H, Dh = 16, 80, 512, 32, 128
M = B * S
C = (Dh ** -0.5) * math.log2(math.e)
HQ = 4
QH = H // HQ
NQ = 2 * QH
XC = 4
XR = M // XC
NSLOT = 4
CB = 8
LAST_CHUNKS = (4, 4, 4, 2, 2)
TAIL_PIECES = (96, 48, 16)
N_OUT_SEMS = 1 + (len(LAST_CHUNKS) - 1) + len(TAIL_PIECES)


def _chunks(sizes):
    out, b0 = [], 0
    for n in sizes:
        out.append((b0, n))
        b0 += n
    assert b0 == B
    return out


def _even(cb):
    return _chunks([cb] * (B // cb))


def _rows(ch):
    b0, nb = ch
    return slice(b0 * S, (b0 + nb) * S)


def _kernel(ax, ak, av, awq, awo, bx, bk, bv, bwq, bwo, out,
            x_buf, kv_buf, wq_buf, wo_buf, q_scr, o_scr, acc, stage,
            sem_pro, sem_kv, sem_wq, sem_wo, sem_out):
    cp = pltpu.make_async_copy

    def xa_copy(c):
        return cp(ax.at[c * XR:(c + 1) * XR], x_buf.at[0, c * XR:(c + 1) * XR], sem_pro.at[c])

    def xb_copy():
        return cp(bx, x_buf.at[1], sem_pro.at[0])

    def wq0_first():
        return cp(awq.at[:, 0:Dh], wq_buf.at[0, :, 0:Dh], sem_pro.at[XC])

    def wq0_rest():
        return cp(awq.at[:, Dh:HQ * Dh], wq_buf.at[0, :, Dh:HQ * Dh], sem_pro.at[XC + 1])

    def by_half(q, fn):
        if isinstance(q, int):
            if q < NQ:
                fn(q // QH, q % QH)
            return

        @pl.when(q < QH)
        def _():
            fn(0, q)

        @pl.when(jnp.logical_and(q >= QH, q < NQ))
        def _():
            fn(1, q - QH)

    def slot_of(q):
        return q % NSLOT if isinstance(q, int) else lax.bitwise_and(q, NSLOT - 1)

    def half_of(q):
        return jnp.where(q >= QH, 1, 0)

    def start_kvo(q):
        sl = slot_of(q)

        def fn(half, g):
            cp((ak, bk)[half].at[:, pl.ds(g * HQ, HQ)], kv_buf.at[sl, 0], sem_kv.at[sl]).start()
            cp((av, bv)[half].at[:, pl.ds(g * HQ, HQ)], kv_buf.at[sl, 1], sem_kv.at[sl]).start()
            cp((awo, bwo)[half].at[pl.ds(g * (HQ * Dh), HQ * Dh), :], wo_buf.at[sl], sem_wo.at[sl]).start()
        by_half(q, fn)

    def start_wq(q):
        sl = slot_of(q)

        def fn(half, g):
            cp((awq, bwq)[half].at[:, pl.ds(g * (HQ * Dh), HQ * Dh)], wq_buf.at[sl], sem_wq.at[sl]).start()
        by_half(q, fn)

    def wait_kvo(q):
        sl = slot_of(q)
        cp(kv_buf.at[sl], kv_buf.at[sl], sem_kv.at[sl]).wait()
        cp(wo_buf.at[sl], wo_buf.at[sl], sem_wo.at[sl]).wait()

    def wait_wq(q):
        sl = slot_of(q)
        cp(wq_buf.at[sl], wq_buf.at[sl], sem_wq.at[sl]).wait()

    def qproj(sx, sl, i, rs):
        q_scr[sl, i, rs, :] = jnp.dot(x_buf[sx, rs, :], wq_buf[sl, :, pl.ds(i * Dh, Dh)],
                                      preferred_element_type=jnp.float32).astype(jnp.bfloat16)

    def oproj(osl, sl, i, rs):
        return jnp.dot(o_scr[osl, rs, :], wo_buf[sl, pl.ds(i * Dh, Dh), :], preferred_element_type=jnp.float32)

    def scores(sl, i, ch):
        b0, nb = ch
        scs = [lax.dot_general(q_scr[sl, i, b * S:(b + 1) * S, :], kv_buf[sl, 0, b, i],
                               (((1,), (1,)), ((), ())), preferred_element_type=jnp.float32)
               for b in range(b0, b0 + nb)]
        ps, ls = [], []
        for sc in scs:
            m = jnp.max(sc, axis=-1, keepdims=True)
            p = jnp.exp2((sc - m) * C)
            ls.append(jnp.sum(p, axis=-1, keepdims=True))
            ps.append(p.astype(jnp.bfloat16))
        return ps, ls

    def pv(ps, ls, osl, sl, i, ch):
        b0, nb = ch
        os_ = [jnp.dot(ps[k], kv_buf[sl, 1, b0 + k, i], preferred_element_type=jnp.float32) for k in range(nb)]
        for k in range(nb):
            o = os_[k] * pl.reciprocal(ls[k], approx=True)
            o_scr[osl, (b0 + k) * S:(b0 + k + 1) * S, :] = o.astype(jnp.bfloat16)

    def accumulate(it, osl):
        sl, i, ch, sa = it['att']
        rs = _rows(ch)
        if it.get('final'):
            r0 = rs.start
            for n in it['final']:
                r = slice(r0, r0 + n)
                r0 += n
                val = acc[sa, r, :] + oproj(osl, sl, i, r)
                stage[sa, r, :] = val.astype(jnp.bfloat16)
                cpy = cp(stage.at[sa, r], out.at[r, pl.ds(D, D)], sem_out.at[1 + len(it['copies'])])
                cpy.start()
                it['copies'].append(cpy)
            return
        val = oproj(osl, sl, i, rs)
        first = it.get('first')
        if first is None:
            val = acc[sa, rs, :] + val
        else:
            val = jnp.where(first, 0.0, acc[sa, rs, :]) + val
        acc[sa, rs, :] = val
        if it.get('stage'):
            stage[sa, rs, :] = val.astype(jnp.bfloat16)

    def block(items):
        n = len(items)
        sc = {}

        def S_(j):
            sl, i, ch, _ = items[j]['att']
            sc[j] = scores(sl, i, ch)

        def P_(j):
            sl, i, ch, _ = items[j]['att']
            ps, ls = sc.pop(j)
            pv(ps, ls, j % 2, sl, i, ch)

        def O_(j):
            accumulate(items[j], j % 2)

        def Q_(j):
            qproj(*items[j]['q'])

        if items[0]['q'] is not None:
            for j in range(n):
                S_(j)
                if j < n - 1:
                    Q_(j)
                    P_(j)
                    if j > 0:
                        O_(j - 1)
                else:
                    O_(j - 1)
                    P_(j)
                    Q_(j)
                    O_(j)
        else:
            S_(0)
            for j in range(n):
                if j + 1 < n:
                    S_(j + 1)
                P_(j)
                if j > 0:
                    O_(j - 1)
            O_(n - 1)

    def xr(c):
        return slice(c * XR, (c + 1) * XR)

    def first_waves(w, carry):
        @pl.when(w == 0)
        def _():
            wq0_first().start()
            xa_copy(0).start()

        @pl.when(w == 1)
        def _():
            wq0_rest().start()
            xa_copy(1).start()
        return carry
    lax.fori_loop(0, 2, first_waves, 0)

    wq0_first().wait()
    xa_copy(0).wait()
    xa_copy(2).start()
    xa_copy(3).start()
    qproj(0, 0, 0, xr(0))

    wq0_rest().wait()
    start_wq(1)
    for i in range(1, HQ):
        qproj(0, 0, i, xr(0))

    xa_copy(1).wait()
    xa_copy(2).wait()
    start_kvo(0)
    start_wq(2)
    for c in (1, 2):
        for i in range(HQ):
            qproj(0, 0, i, xr(c))

    xa_copy(3).wait()
    wait_wq(1)
    start_kvo(1)
    start_wq(3)
    start_kvo(2)
    for i in range(HQ):
        qproj(0, 0, i, xr(3))
    for c in range(XC):
        for i in range(HQ):
            qproj(0, 1, i, xr(c))
    start_kvo(3)
    start_wq(4)
    start_wq(5)

    def quad_body(r, carry):
        wait_kvo(r)
        wait_wq(r + 2)
        block([dict(att=(r, i, ch, 0), q=(0, r + 2, i, _rows(ch)), first=(r == 0) if i == 0 else None)
               for i in range(HQ) for ch in _even(CB)])
        start_kvo(r + NSLOT)
        start_wq(r + 2 + NSLOT)
        return carry
    lax.fori_loop(0, 2, quad_body, 0)

    def main_body(m, carry):
        q0 = 2 + 2 * m

        @pl.when(q0 + 2 == QH)
        def _():
            xb_copy().wait()
        wait_kvo(q0)
        wait_kvo(q0 + 1)
        wait_wq(q0 + 2)
        wait_wq(q0 + 3)

        @pl.when(q0 == QH)
        def _():
            cp(stage.at[0], out.at[:, pl.ds(0, D)], sem_out.at[0]).start()
        items = []
        for d in range(2):
            qq = q0 + d
            sl, sln = slot_of(qq), slot_of(qq + 2)
            sa, sx = half_of(qq), half_of(qq + 2)
            for i in range(HQ):
                for ch in _even(CB):
                    items.append(dict(att=(sl, i, ch, sa), q=(sx, sln, i, _rows(ch)),
                                      first=(qq == QH) if (d == 0 and i == 0) else None,
                                      stage=(d == 1 and i == HQ - 1)))
        block(items)
        start_kvo(q0 + NSLOT)
        start_kvo(q0 + 1 + NSLOT)
        start_wq(q0 + 2 + NSLOT)
        start_wq(q0 + 3 + NSLOT)

        @pl.when(m == 0)
        def _():
            xb_copy().start()
        return carry
    lax.fori_loop(0, (NQ - 4) // 2, main_body, 0)

    wait_kvo(NQ - 2)
    wait_kvo(NQ - 1)
    copies = []
    s14, s15 = (NQ - 2) % NSLOT, (NQ - 1) % NSLOT
    items = [dict(att=(s14, i, ch, 1), q=None) for i in range(HQ) for ch in _even(CB)]
    last_chunks = _chunks(LAST_CHUNKS)
    for k, ch in enumerate(last_chunks):
        for i in range(HQ):
            final = None
            if i == HQ - 1:
                final = TAIL_PIECES if k == len(last_chunks) - 1 else (ch[1] * S,)
            items.append(dict(att=(s15, i, ch, 1), q=None, final=final, copies=copies))
    block(items)
    for cpy in copies:
        cpy.wait()
    cp(stage.at[0], out.at[:, pl.ds(0, D)], sem_out.at[0]).wait()


@jax.jit
def pallas_concat_heads__mha_block_cached__mha_block_cached__near_ridge_kernel(
    A_x: jax.Array,
    A_k_cache: jax.Array,
    A_v_cache: jax.Array,
    A_wq: jax.Array,
    A_wo: jax.Array,
    B_x: jax.Array,
    B_k_cache: jax.Array,
    B_v_cache: jax.Array,
    B_wq: jax.Array,
    B_wo: jax.Array,
):
    assert sum(TAIL_PIECES) == LAST_CHUNKS[-1] * S
    any_spec = pl.BlockSpec(memory_space=pl.ANY)
    out = pl.pallas_call(
        _kernel,
        in_specs=[any_spec] * 10,
        out_specs=any_spec,
        out_shape=jax.ShapeDtypeStruct((M, 2 * D), jnp.bfloat16),
        scratch_shapes=[
            pltpu.VMEM((2, M, D), jnp.bfloat16),
            pltpu.VMEM((NSLOT, 2, B, HQ, S, Dh), jnp.bfloat16),
            pltpu.VMEM((NSLOT, D, HQ * Dh), jnp.bfloat16),
            pltpu.VMEM((NSLOT, HQ * Dh, D), jnp.bfloat16),
            pltpu.VMEM((NSLOT, HQ, M, Dh), jnp.bfloat16),
            pltpu.VMEM((2, M, Dh), jnp.bfloat16),
            pltpu.VMEM((2, M, D), jnp.float32),
            pltpu.VMEM((2, M, D), jnp.bfloat16),
            pltpu.SemaphoreType.DMA((XC + 2,)),
            pltpu.SemaphoreType.DMA((NSLOT,)),
            pltpu.SemaphoreType.DMA((NSLOT,)),
            pltpu.SemaphoreType.DMA((NSLOT,)),
            pltpu.SemaphoreType.DMA((N_OUT_SEMS,)),
        ],
        compiler_params=pltpu.CompilerParams(
            vmem_limit_bytes=64 * 1024 * 1024,
            disable_bounds_checks=True,
            disable_semaphore_checks=True,
        ),
    )(A_x.reshape(M, D), A_k_cache, A_v_cache, A_wq, A_wo, B_x.reshape(M, D), B_k_cache, B_v_cache, B_wq, B_wo)
    return out.reshape(B, S, 2 * D)
```

```python
import math

import jax
import jax.numpy as jnp
from jax import lax
from jax.experimental import pallas as pl
from jax.experimental.pallas import tpu as pltpu

B, S, D, H, Dh = 16, 80, 512, 32, 128
M = B * S
C = (Dh ** -0.5) * math.log2(math.e)
HQ = 4
QH = H // HQ
NQ = 2 * QH
XC = 4
XR = M // XC
NSLOT = 4
CB = 8
LAST_CHUNKS = (4, 4, 4, 2, 2)
TAIL_PIECES = (96, 48, 16)
N_OUT_SEMS = 1 + (len(LAST_CHUNKS) - 1) + len(TAIL_PIECES)


def _chunks(sizes):
    out, b0 = [], 0
    for n in sizes:
        out.append((b0, n))
        b0 += n
    assert b0 == B
    return out


def _even(cb):
    return _chunks([cb] * (B // cb))


def _rows(ch):
    b0, nb = ch
    return slice(b0 * S, (b0 + nb) * S)


def _kernel(ax, ak, av, awq, awo, bx, bk, bv, bwq, bwo, out,
            x_buf, kv_buf, wq_buf, wo_buf, q_scr, o_scr, acc, stage,
            sem_pro, sem_kv, sem_wq, sem_wo, sem_out):
    cp = pltpu.make_async_copy

    def xa_copy(c):
        return cp(ax.at[c * XR:(c + 1) * XR], x_buf.at[0, c * XR:(c + 1) * XR], sem_pro.at[c])

    def xb_copy():
        return cp(bx, x_buf.at[1], sem_pro.at[0])

    def wq0_first():
        return cp(awq.at[:, 0:Dh], wq_buf.at[0, :, 0:Dh], sem_pro.at[XC])

    def wq0_rest():
        return cp(awq.at[:, Dh:HQ * Dh], wq_buf.at[0, :, Dh:HQ * Dh], sem_pro.at[XC + 1])

    def by_half(q, fn):
        if isinstance(q, int):
            if q < NQ:
                fn(q // QH, q % QH)
            return

        @pl.when(q < QH)
        def _():
            fn(0, q)

        @pl.when(jnp.logical_and(q >= QH, q < NQ))
        def _():
            fn(1, q - QH)

    def slot_of(q):
        return q % NSLOT if isinstance(q, int) else lax.bitwise_and(q, NSLOT - 1)

    def half_of(q):
        return jnp.where(q >= QH, 1, 0)

    def start_kvo(q):
        sl = slot_of(q)

        def fn(half, g):
            cp((ak, bk)[half].at[:, pl.ds(g * HQ, HQ)], kv_buf.at[sl, 0], sem_kv.at[sl]).start()
            cp((av, bv)[half].at[:, pl.ds(g * HQ, HQ)], kv_buf.at[sl, 1], sem_kv.at[sl]).start()
            cp((awo, bwo)[half].at[pl.ds(g * (HQ * Dh), HQ * Dh), :], wo_buf.at[sl], sem_wo.at[sl]).start()
        by_half(q, fn)

    def start_wq(q):
        sl = slot_of(q)

        def fn(half, g):
            cp((awq, bwq)[half].at[:, pl.ds(g * (HQ * Dh), HQ * Dh)], wq_buf.at[sl], sem_wq.at[sl]).start()
        by_half(q, fn)

    def wait_kvo(q):
        sl = slot_of(q)
        cp(kv_buf.at[sl], kv_buf.at[sl], sem_kv.at[sl]).wait()
        cp(wo_buf.at[sl], wo_buf.at[sl], sem_wo.at[sl]).wait()

    def wait_wq(q):
        sl = slot_of(q)
        cp(wq_buf.at[sl], wq_buf.at[sl], sem_wq.at[sl]).wait()

    def qproj(sx, sl, i, rs):
        q_scr[sl, i, rs, :] = jnp.dot(x_buf[sx, rs, :], wq_buf[sl, :, pl.ds(i * Dh, Dh)],
                                      preferred_element_type=jnp.float32).astype(jnp.bfloat16)

    def oproj(osl, sl, i, rs):
        return jnp.dot(o_scr[osl, rs, :], wo_buf[sl, pl.ds(i * Dh, Dh), :], preferred_element_type=jnp.float32)

    def scores(sl, i, ch):
        b0, nb = ch
        scs = [lax.dot_general(q_scr[sl, i, b * S:(b + 1) * S, :], kv_buf[sl, 0, b, i],
                               (((1,), (1,)), ((), ())), preferred_element_type=jnp.float32)
               for b in range(b0, b0 + nb)]
        ps, ls = [], []
        for sc in scs:
            m = jnp.max(sc, axis=-1, keepdims=True)
            p = jnp.exp2((sc - m) * C)
            ls.append(jnp.sum(p, axis=-1, keepdims=True))
            ps.append(p.astype(jnp.bfloat16))
        return ps, ls

    def pv(ps, ls, osl, sl, i, ch):
        b0, nb = ch
        os_ = [jnp.dot(ps[k], kv_buf[sl, 1, b0 + k, i], preferred_element_type=jnp.float32) for k in range(nb)]
        for k in range(nb):
            o = os_[k] * pl.reciprocal(ls[k], approx=True)
            o_scr[osl, (b0 + k) * S:(b0 + k + 1) * S, :] = o.astype(jnp.bfloat16)

    def accumulate(it, osl):
        sl, i, ch, sa = it['att']
        rs = _rows(ch)
        if it.get('final'):
            r0 = rs.start
            for n in it['final']:
                r = slice(r0, r0 + n)
                r0 += n
                val = acc[sa, r, :] + oproj(osl, sl, i, r)
                stage[sa, r, :] = val.astype(jnp.bfloat16)
                cpy = cp(stage.at[sa, r], out.at[r, pl.ds(D, D)], sem_out.at[1 + len(it['copies'])])
                cpy.start()
                it['copies'].append(cpy)
            return
        val = oproj(osl, sl, i, rs)
        first = it.get('first')
        if first is None:
            val = acc[sa, rs, :] + val
        else:
            val = jnp.where(first, 0.0, acc[sa, rs, :]) + val
        acc[sa, rs, :] = val
        if it.get('stage'):
            stage[sa, rs, :] = val.astype(jnp.bfloat16)

    def block(items):
        n = len(items)
        sc = {}

        def S_(j):
            sl, i, ch, _ = items[j]['att']
            sc[j] = scores(sl, i, ch)

        def P_(j):
            sl, i, ch, _ = items[j]['att']
            ps, ls = sc.pop(j)
            pv(ps, ls, j % 2, sl, i, ch)

        def O_(j):
            accumulate(items[j], j % 2)

        def Q_(j):
            qproj(*items[j]['q'])

        if items[0]['q'] is not None:
            for j in range(n):
                S_(j)
                if j < n - 1:
                    Q_(j)
                    P_(j)
                    if j > 0:
                        O_(j - 1)
                else:
                    O_(j - 1)
                    P_(j)
                    Q_(j)
                    O_(j)
        else:
            S_(0)
            for j in range(n):
                if j + 1 < n:
                    S_(j + 1)
                P_(j)
                if j > 0:
                    O_(j - 1)
            O_(n - 1)

    def prologue():
        def xr(c):
            return slice(c * XR, (c + 1) * XR)

        def first_waves(w, carry):
            @pl.when(w == 0)
            def _():
                wq0_first().start()
                xa_copy(0).start()

            @pl.when(w == 1)
            def _():
                wq0_rest().start()
                xa_copy(1).start()
            return carry
        lax.fori_loop(0, 2, first_waves, 0)

        wq0_first().wait()
        xa_copy(0).wait()
        xa_copy(2).start()
        xa_copy(3).start()
        qproj(0, 0, 0, xr(0))

        wq0_rest().wait()
        start_wq(1)
        for i in range(1, HQ):
            qproj(0, 0, i, xr(0))

        xa_copy(1).wait()
        xa_copy(2).wait()
        start_kvo(0)
        start_wq(2)
        for c in (1, 2):
            for i in range(HQ):
                qproj(0, 0, i, xr(c))

        xa_copy(3).wait()
        wait_wq(1)
        start_kvo(1)
        start_wq(3)
        start_kvo(2)
        for i in range(HQ):
            qproj(0, 0, i, xr(3))
        for c in range(XC):
            for i in range(HQ):
                qproj(0, 1, i, xr(c))
        start_kvo(3)
        start_wq(4)
        start_wq(5)

    def quad_block(r):
        wait_kvo(r)
        wait_wq(r + 2)
        block([dict(att=(r, i, ch, 0), q=(0, r + 2, i, _rows(ch)), first=(r == 0) if i == 0 else None)
               for i in range(HQ) for ch in _even(CB)])
        start_kvo(r + NSLOT)
        start_wq(r + 2 + NSLOT)

    def main_block(m):
        q0 = 2 + 2 * m

        @pl.when(q0 + 2 == QH)
        def _():
            xb_copy().wait()
        wait_kvo(q0)
        wait_kvo(q0 + 1)
        wait_wq(q0 + 2)
        wait_wq(q0 + 3)

        @pl.when(q0 == QH)
        def _():
            cp(stage.at[0], out.at[:, pl.ds(0, D)], sem_out.at[0]).start()
        items = []
        for d in range(2):
            qq = q0 + d
            sl, sln = slot_of(qq), slot_of(qq + 2)
            sa, sx = half_of(qq), half_of(qq + 2)
            for i in range(HQ):
                for ch in _even(CB):
                    items.append(dict(att=(sl, i, ch, sa), q=(sx, sln, i, _rows(ch)),
                                      first=(qq == QH) if (d == 0 and i == 0) else None,
                                      stage=(d == 1 and i == HQ - 1)))
        block(items)
        start_kvo(q0 + NSLOT)
        start_kvo(q0 + 1 + NSLOT)
        start_wq(q0 + 2 + NSLOT)
        start_wq(q0 + 3 + NSLOT)

        @pl.when(m == 0)
        def _():
            xb_copy().start()

    def last_block():
        wait_kvo(NQ - 2)
        wait_kvo(NQ - 1)
        copies = []
        s14, s15 = (NQ - 2) % NSLOT, (NQ - 1) % NSLOT
        items = [dict(att=(s14, i, ch, 1), q=None) for i in range(HQ) for ch in _even(CB)]
        last_chunks = _chunks(LAST_CHUNKS)
        for k, ch in enumerate(last_chunks):
            for i in range(HQ):
                final = None
                if i == HQ - 1:
                    final = TAIL_PIECES if k == len(last_chunks) - 1 else (ch[1] * S,)
                items.append(dict(att=(s15, i, ch, 1), q=None, final=final, copies=copies))
        block(items)
        for cpy in copies:
            cpy.wait()
        cp(stage.at[0], out.at[:, pl.ds(0, D)], sem_out.at[0]).wait()

    n_main = (NQ - 4) // 2

    def phase(t, carry):
        @pl.when(t == 0)
        def _():
            prologue()

        @pl.when(jnp.logical_and(t >= 1, t < 3))
        def _():
            quad_block(t - 1)

        @pl.when(jnp.logical_and(t >= 3, t < 3 + n_main))
        def _():
            main_block(t - 3)

        @pl.when(t == 3 + n_main)
        def _():
            last_block()
        return carry
    lax.fori_loop(0, 4 + n_main, phase, 0)


@jax.jit
def pallas_concat_heads__mha_block_cached__mha_block_cached__near_ridge_kernel(
    A_x: jax.Array,
    A_k_cache: jax.Array,
    A_v_cache: jax.Array,
    A_wq: jax.Array,
    A_wo: jax.Array,
    B_x: jax.Array,
    B_k_cache: jax.Array,
    B_v_cache: jax.Array,
    B_wq: jax.Array,
    B_wo: jax.Array,
):
    assert sum(TAIL_PIECES) == LAST_CHUNKS[-1] * S
    any_spec = pl.BlockSpec(memory_space=pl.ANY)
    out = pl.pallas_call(
        _kernel,
        in_specs=[any_spec] * 10,
        out_specs=any_spec,
        out_shape=jax.ShapeDtypeStruct((M, 2 * D), jnp.bfloat16),
        scratch_shapes=[
            pltpu.VMEM((2, M, D), jnp.bfloat16),
            pltpu.VMEM((NSLOT, 2, B, HQ, S, Dh), jnp.bfloat16),
            pltpu.VMEM((NSLOT, D, HQ * Dh), jnp.bfloat16),
            pltpu.VMEM((NSLOT, HQ * Dh, D), jnp.bfloat16),
            pltpu.VMEM((NSLOT, HQ, M, Dh), jnp.bfloat16),
            pltpu.VMEM((2, M, Dh), jnp.bfloat16),
            pltpu.VMEM((2, M, D), jnp.float32),
            pltpu.VMEM((2, M, D), jnp.bfloat16),
            pltpu.SemaphoreType.DMA((XC + 2,)),
            pltpu.SemaphoreType.DMA((NSLOT,)),
            pltpu.SemaphoreType.DMA((NSLOT,)),
            pltpu.SemaphoreType.DMA((NSLOT,)),
            pltpu.SemaphoreType.DMA((N_OUT_SEMS,)),
        ],
        compiler_params=pltpu.CompilerParams(
            vmem_limit_bytes=64 * 1024 * 1024,
            disable_bounds_checks=True,
            disable_semaphore_checks=True,
        ),
    )(A_x.reshape(M, D), A_k_cache, A_v_cache, A_wq, A_wo, B_x.reshape(M, D), B_k_cache, B_v_cache, B_wq, B_wo)
    return out.reshape(B, S, 2 * D)
```
